```python
import os as _os
_os.environ.setdefault("JAX_PLATFORMS", "cpu")
import jax
import jax.numpy as jnp

def _softmax(x, axis=-1):
    return jax.nn.softmax(x, axis=axis)
def _gelu(x):
    return jax.nn.gelu(x, approximate=True)
def _silu(x):
    return jax.nn.silu(x)
def _sigmoid(x):
    return jax.nn.sigmoid(x)
def _layernorm(x, axis=-1, eps=1e-5):
    m = jnp.mean(x, axis=axis, keepdims=True)
    v = jnp.var(x, axis=axis, keepdims=True)
    return (x - m) / jnp.sqrt(v + eps)
def _scatter_add(tgt, idx, src, axis=0):
    return tgt.at[idx].add(src)
def _segment_sum(src, seg, n):
    return jax.ops.segment_sum(src, seg, n)
class _Rng:
    def __init__(self, key):
        self._k = key
    def _next(self):
        self._k, sub = jax.random.split(self._k)
        return sub
    def normal(self, shape):
        return jax.random.normal(self._next(), shape, dtype=jnp.bfloat16)
    def randint(self, lo, hi, shape):
        return jax.random.randint(self._next(), shape, lo, hi, dtype=jnp.int32)
    def uniform(self, shape, lo=0.0, hi=1.0):
        return jax.random.uniform(self._next(), shape, jnp.bfloat16, lo, hi)
    def permutation(self, n):
        return jax.random.permutation(self._next(), n)


kernel_name = 'standalone__dcn_v2_cross__recsys'

def setup_inputs():
    _rng = _Rng(jax.random.key(int.from_bytes(__import__("os").urandom(4), "little")))
    _w = (lambda a: (lambda t: t.astype(jnp.bfloat16) if jnp.issubdtype(t.dtype, jnp.floating) else t)(jnp.asarray(a)))
    B, F, D, L = 4096, 26, 128, 6
    Din = min(F * D, 1024)
    return {
        "x0": _w((lambda *s: _rng.normal(s) * 0.05)(B, Din)),
        "ws": _w((lambda *s: _rng.normal(s) * 0.05)(L, Din, Din)),
        "bs": _w((lambda *s: _rng.normal(s) * 0.05)(L, Din)),
    }

def reference(x0, ws, bs):
    x = x0
    for l in range(ws.shape[0]):
        x = x0 * (x @ ws[l] + bs[l]) + x
    return x
```

```python
import functools
import jax, jax.numpy as jnp
from jax import lax
from jax.experimental import pallas as pl
from jax.experimental.pallas import tpu as pltpu

F32 = jnp.float32; BF = jnp.bfloat16; U32 = jnp.uint32

SDEF = {1: [(1, 0), (1, 3)], 2: [(1, 2), (1, 3)], 3: [(1, 0)], 4: [(1, 3)], 5: [(1, 0), (1, 1)], 6: [(1, 2), (-1, 0)], 7: [(1, 1), (-1, 3)]}
TDEF = {1: [(1, 0), (1, 3)], 2: [(1, 0)], 3: [(1, 1), (-1, 3)], 4: [(1, 2), (-1, 0)], 5: [(1, 3)], 6: [(1, 0), (1, 1)], 7: [(1, 2), (1, 3)]}

def lin(terms):
    terms = sorted(terms, key=lambda t: -t[0])
    acc = None
    for s, v in terms:
        if acc is None:
            assert s == 1
            acc = v
        else:
            acc = acc + v if s == 1 else acc - v
    return acc

def quad(X, q):
    r, c = divmod(q, 2)
    return [X[2*r + (k // 2)][2*c + (k % 2)] for k in range(4)]

def layer(A, Z, bias, getT, pre, order):
    def level2(S, i1):
        ops = {}
        def M(i, j):
            if i not in ops:
                ops[i] = lin([(s * s2, v) for s, q in SDEF[i] for s2, v in S[q]]).astype(BF)
            return jnp.dot(ops[i], getT(i1, i, j), preferred_element_type=F32)
        out = [[None, None] for _ in range(4)]
        for j in range(2):
            M1 = M(1, j)
            P = M1 + M(7, j)
            Q = M1 + M(6, j)
            M2 = M(2, j)
            M4 = M(4, j)
            out[2][j] = M2 + M4
            P = P + M4
            Q = Q - M2
            M3 = M(3, j)
            M5 = M(5, j)
            out[1][j] = M3 + M5
            out[0][j] = P - M5
            out[3][j] = Q + M3
        return out
    def r(i):
        pre(i)
        S = [[(s, quad(A, q)[k]) for s, q in SDEF[i]] for k in range(4)]
        return level2(S, i)
    add = lambda X, Y: [[X[k][j] + Y[k][j] for j in range(2)] for k in range(4)]
    sub = lambda X, Y: [[X[k][j] - Y[k][j] for j in range(2)] for k in range(4)]
    N = [[None] * 4 for _ in range(4)]
    def F(q, Cq):
        r_, c_ = divmod(q, 2)
        for k in range(4):
            R, C = 2*r_ + k // 2, 2*c_ + k % 2
            c = jnp.concatenate(Cq[k], axis=1)
            N[R][C] = Z[R][C] * (c + bias[C]) + A[R][C]
    if order == 0:
        M4 = r(4); M2 = r(2); F(2, add(M2, M4))
        C11 = add(M4, r(7)); M1 = r(1); C11 = add(C11, M1); C22 = sub(M1, M2)
        M5 = r(5); F(0, sub(C11, M5))
        M3 = r(3); F(1, add(M3, M5)); C22 = add(C22, M3)
        F(3, add(C22, r(6)))
    else:
        M6 = r(6); M3 = r(3); C22 = add(M6, M3)
        M5 = r(5); F(1, add(M3, M5))
        M1 = r(1); C22 = add(C22, M1); C11 = sub(M1, M5)
        M2 = r(2); F(3, sub(C22, M2))
        M4 = r(4); F(2, add(M2, M4)); C11 = add(C11, M4)
        F(0, add(C11, r(7)))
    return N

def make(tm=256, nsb=2, mode='mem', prep_rows=32, split=False):
    rs = tm // 4
    ts = tm * nsb

    def kernel(x0_hbm, w_hbm, b_hbm, o_hbm, xbuf, obuf, wbuf, t_ref, braw, bf32, xs32, x0s, os16,
               xsem, osem, wsem, ssem):
        L, D, _ = wbuf.shape
        B = x0_hbm.shape[0]
        nb = B // tm
        cs = D // 4

        def xcopy(i, slot):
            return pltpu.make_async_copy(x0_hbm.at[pl.ds(pl.multiple_of(i * tm, tm), tm)], xbuf.at[slot], xsem.at[slot])
        def ocopy(i, slot):
            return pltpu.make_async_copy(obuf.at[slot], o_hbm.at[pl.ds(pl.multiple_of(i * tm, tm), tm)], osem.at[slot])
        def wcopy(l):
            return pltpu.make_async_copy(w_hbm.at[l], wbuf.at[l], wsem.at[l])
        bcopy = pltpu.make_async_copy(b_hbm, braw, ssem.at[0])
        x0copy = pltpu.make_async_copy(x0_hbm.at[pl.ds(0, ts)], x0s, ssem.at[1])
        o0copy = pltpu.make_async_copy(os16, o_hbm.at[pl.ds(0, ts)], ssem.at[2])

        bcopy.start()
        x0copy.start()
        def _ws(l, c):
            wcopy(l).start()
            return c
        lax.fori_loop(0, L, _ws, 0)
        xcopy(nsb, nsb % 2).start()

        bcopy.wait()
        bf32[0:L, :] = braw[...].astype(F32)
        x0copy.wait()
        xs32[...] = x0s[...].astype(F32)

        def tidx(l, i, i2, j):
            return ((l * 7 + i - 1) * 7 + i2 - 1) * 2 + j

        def prep1(l, i):
            pr = prep_rows
            for j in range(2):
                for r0 in range(0, cs, pr):
                    def wt(R, C):
                        return wbuf[l, R*cs + r0:R*cs + r0 + pr, C*cs + j*128:C*cs + (j+1)*128].astype(F32)
                    S = [lin([(s, wt(2*(q//2) + k//2, 2*(q % 2) + k % 2)) for s, q in TDEF[i]]) for k in range(4)]
                    for i2 in range(1, 8):
                        v = lin([(s, S[q]) for s, q in TDEF[i2]]).astype(BF)
                        t_ref[tidx(l, i, i2, j), r0//2:(r0 + pr)//2, :] = pltpu.bitcast(v, U32)

        def start_body(l, carry):
            wcopy(l).wait()
            brow = bf32[pl.ds(l, 1), :]
            bias = [brow[:, C*cs:(C+1)*cs] for C in range(4)]
            if mode == 'mem':
                getT = lambda i, i2, j: pltpu.bitcast(t_ref[tidx(l, i, i2, j)], BF)
                pre = lambda i: prep1(l, i)
            else:
                TS = {}
                def pre(i):
                    def wt(R, C):
                        return wbuf[l, R*cs:(R+1)*cs, C*cs:(C+1)*cs].astype(F32)
                    TS[i] = [lin([(s, wt(2*(q//2) + k//2, 2*(q % 2) + k % 2)) for s, q in TDEF[i]]) for k in range(4)]
                def getT(i, i2, j):
                    v = lin([(s, TS[i][q][:, j*128:(j+1)*128]) for s, q in TDEF[i2]]).astype(BF)
                    t_ref[tidx(l, i, i2, j)] = pltpu.bitcast(v, U32)
                    return v
            if split:
                for h in range(nsb):
                    o = h * tm
                    Z = [[x0s[o + R*rs:o + (R+1)*rs, C*cs:(C+1)*cs].astype(F32) for C in range(4)] for R in range(4)]
                    A = [[xs32[o + R*rs:o + (R+1)*rs, C*cs:(C+1)*cs] for C in range(4)] for R in range(4)]
                    if h == 0:
                        N = layer(A, Z, bias, getT, pre, 0)
                    else:
                        N = layer(A, Z, bias, lambda i, i2, j: pltpu.bitcast(t_ref[tidx(l, i, i2, j)], BF), lambda i: None, 0)
                    for R in range(4):
                        for C in range(4):
                            xs32[o + R*rs:o + (R+1)*rs, C*cs:(C+1)*cs] = N[R][C]
            else:
                r2 = ts // 4
                Z = [[x0s[R*r2:(R+1)*r2, C*cs:(C+1)*cs].astype(F32) for C in range(4)] for R in range(4)]
                A = [[xs32[R*r2:(R+1)*r2, C*cs:(C+1)*cs] for C in range(4)] for R in range(4)]
                N = layer(A, Z, bias, getT, pre, 0)
                for R in range(4):
                    for C in range(4):
                        xs32[R*r2:(R+1)*r2, C*cs:(C+1)*cs] = N[R][C]
            return carry
        lax.fori_loop(0, L, start_body, 0)
        os16[...] = xs32[...].astype(BF)
        o0copy.start()

        def block(xr, orf):
            Z = [[xr[R*rs:(R+1)*rs, C*cs:(C+1)*cs].astype(F32) for C in range(4)] for R in range(4)]
            A = Z
            for l in range(L):
                bias = [bf32[l:l+1, C*cs:(C+1)*cs] for C in range(4)]
                A = layer(A, Z, bias, lambda i, i2, j: pltpu.bitcast(t_ref[tidx(l, i, i2, j)], BF), lambda i: None, l % 2)
            for R in range(4):
                for C in range(4):
                    orf[R*rs:(R+1)*rs, C*cs:(C+1)*cs] = A[R][C].astype(BF)

        def main_body(i, carry):
            slot = i % 2
            xcopy(i, slot).wait()
            @pl.when(i + 1 < nb)
            def _():
                xcopy(i + 1, 1 - slot).start()
            @pl.when(i >= nsb + 2)
            def _():
                ocopy(i - 2, slot).wait()
            block(xbuf.at[slot], obuf.at[slot])
            ocopy(i, slot).start()
            return carry
        lax.fori_loop(nsb, nb, main_body, 0)
        o0copy.wait()
        ocopy(nb - 2, (nb - 2) % 2).wait()
        ocopy(nb - 1, (nb - 1) % 2).wait()

    @jax.jit
    def f(x0, ws, bs):
        B, D = x0.shape
        L = ws.shape[0]
        return pl.pallas_call(
            kernel,
            in_specs=[pl.BlockSpec(memory_space=pl.ANY)] * 3,
            out_specs=pl.BlockSpec(memory_space=pl.ANY),
            out_shape=jax.ShapeDtypeStruct((B, D), x0.dtype),
            scratch_shapes=[
                pltpu.VMEM((2, tm, D), BF), pltpu.VMEM((2, tm, D), BF),
                pltpu.VMEM((L, D, D), BF), pltpu.VMEM((L * 98, D // 8, 128), U32),
                pltpu.VMEM((L, D), BF), pltpu.VMEM((8, D), F32),
                pltpu.VMEM((ts, D), F32), pltpu.VMEM((ts, D), BF), pltpu.VMEM((ts, D), BF),
                pltpu.SemaphoreType.DMA((2,)), pltpu.SemaphoreType.DMA((2,)),
                pltpu.SemaphoreType.DMA((L,)), pltpu.SemaphoreType.DMA((3,)),
            ],
            compiler_params=pltpu.CompilerParams(vmem_limit_bytes=100 * 1024 * 1024),
        )(x0, ws, bs)
    return f


_impl = make(256, 2, 'mem', 32, False)


@jax.jit
def pallas_standalone__dcn_v2_cross__recsys_kernel(x0: jax.Array, ws: jax.Array, bs: jax.Array):
    return _impl(x0, ws, bs)
```

```python
import functools

import jax
import jax.numpy as jnp
from jax import lax
from jax.experimental import pallas as pl
from jax.experimental.pallas import tpu as pltpu

F32 = jnp.float32
BF16 = jnp.bfloat16
U32 = jnp.uint32

TM = 256
G = 4
PREP_ROWS = 32
LANES = 128

_LHS = {1: ((1, 0), (1, 3)), 2: ((1, 2), (1, 3)), 3: ((1, 0),), 4: ((1, 3),),
        5: ((1, 0), (1, 1)), 6: ((1, 2), (-1, 0)), 7: ((1, 1), (-1, 3))}
_RHS = {1: ((1, 0), (1, 3)), 2: ((1, 0),), 3: ((1, 1), (-1, 3)), 4: ((1, 2), (-1, 0)),
        5: ((1, 3),), 6: ((1, 0), (1, 1)), 7: ((1, 2), (1, 3))}
_OUT = {0: {1: 1, 4: 1, 5: -1, 7: 1}, 1: {3: 1, 5: 1}, 2: {2: 1, 4: 1}, 3: {1: 1, 2: -1, 3: 1, 6: 1}}

_ORDER_X = (4, 2, 7, 1, 5, 3, 6)
_ORDER_Y = (6, 3, 5, 1, 2, 4, 7)
_ORDER_FIRST = (2, 4, 7, 1, 5, 3, 6)


def _signed_sum(terms, add=lambda a, b: a + b, sub=lambda a, b: a - b):
    terms = sorted(terms, key=lambda t: -t[0])
    assert terms[0][0] == 1
    acc = terms[0][1]
    for s, v in terms[1:]:
        acc = add(acc, v) if s == 1 else sub(acc, v)
    return acc


def _combine(order, product, finish, add, sub):
    pending = {q: [] for q in _OUT}
    seen = {q: 0 for q in _OUT}
    for i in order:
        m = product(i)
        for q, coef in _OUT.items():
            if i not in coef:
                continue
            pending[q].append((coef[i], m))
            seen[q] += 1
            if len(pending[q]) == 2:
                pending[q] = [(1, _signed_sum(pending[q], add, sub))]
            if seen[q] == len(coef):
                finish(q, pending[q][0][1])


def _sub_block(q, k):
    return 2 * (q // 2) + k // 2, 2 * (q % 2) + k % 2


def _cross_layer(x, x0, bias, get_t, order, before_product=None, after_quadrant=None):
    ntile = bias[0].shape[1] // LANES

    def inner(terms, i1):
        lhs = {}

        def product(j, i2):
            if i2 not in lhs:
                lhs[i2] = _signed_sum(
                    [(s * s2, v) for s, k in _LHS[i2] for s2, v in terms[k]]).astype(BF16)
            return jnp.dot(lhs[i2], get_t(i1, i2, j), preferred_element_type=F32)

        out = [[None] * ntile for _ in range(4)]
        for j in range(ntile):
            def finish(k, v, j=j):
                out[k][j] = v
            _combine(_ORDER_Y, functools.partial(product, j), finish,
                     lambda a, b: a + b, lambda a, b: a - b)
        return out

    def outer_product(i1):
        if before_product is not None:
            before_product(i1)
        terms = [[(s, x(*_sub_block(q, k))) for s, q in _LHS[i1]] for k in range(4)]
        return inner(terms, i1)

    def zip2(f):
        return lambda a, b: [[f(u, v) for u, v in zip(ra, rb)] for ra, rb in zip(a, b)]

    new = [[None] * 4 for _ in range(4)]

    def outer_finish(q, c):
        for k in range(4):
            r, col = _sub_block(q, k)
            y = jnp.concatenate(c[k], axis=1) + bias[col]
            new[r][col] = x0(r, col) * y + x(r, col)
        if after_quadrant is not None:
            after_quadrant(q, new)

    _combine(order, outer_product, outer_finish, zip2(lambda a, b: a + b), zip2(lambda a, b: a - b))
    return new


def _kernel(x0_hbm, w_hbm, b_hbm, o_hbm,
            xbuf, obuf, wbuf, t_ref, braw, bf32, xs32, x0s, os16,
            xsem, osem, wsem, ssem, qsem):
    n_layers, d, _ = wbuf.shape
    n_blocks = x0_hbm.shape[0] // TM
    cs = d // 4
    hd = d // 2
    ntile = cs // LANES
    rs = TM // 4
    ts = TM * G
    ru = ts // 4
    hm = TM // 2

    def x_copy(i, slot):
        r0 = pl.multiple_of(i * TM, TM)
        return pltpu.make_async_copy(x0_hbm.at[pl.ds(r0, TM)], xbuf.at[slot], xsem.at[slot])

    def o_copy(i, slot, q):
        r0 = pl.multiple_of(i * TM, TM)
        qr, qc = divmod(q, 2)
        return pltpu.make_async_copy(
            obuf.at[slot, pl.ds(qr * hm, hm), pl.ds(qc * hd, hd)],
            o_hbm.at[pl.ds(r0 + qr * hm, hm), pl.ds(qc * hd, hd)],
            osem.at[slot * 4 + q])

    def w_copy(l):
        return pltpu.make_async_copy(w_hbm.at[l], wbuf.at[l], wsem.at[l])

    def w0_quadrant_copy(r, c):
        r0 = pl.multiple_of(r * hd, hd)
        c0 = pl.multiple_of(c * hd, hd)
        return pltpu.make_async_copy(
            w_hbm.at[0, pl.ds(r0, hd), pl.ds(c0, hd)],
            wbuf.at[0, pl.ds(r0, hd), pl.ds(c0, hd)],
            qsem.at[2 * r + c])

    def xs_half_copy(h):
        rows = pl.ds(h * (ts // 2), ts // 2)
        return pltpu.make_async_copy(x0_hbm.at[rows], x0s.at[rows], ssem.at[1 + h])

    b_copy = pltpu.make_async_copy(b_hbm, braw, ssem.at[0])
    os_copy = pltpu.make_async_copy(os16, o_hbm.at[pl.ds(0, ts)], ssem.at[3])

    def loop(lo, hi, fn):
        def body(i, carry):
            fn(i)
            return carry
        lax.fori_loop(lo, hi, body, 0)

    b_copy.start()
    xs_half_copy(1).start()
    loop(0, 2, lambda r: w0_quadrant_copy(r, 0).start())
    xs_half_copy(0).start()
    loop(0, 2, lambda r: w0_quadrant_copy(1 - r, 1).start())
    loop(1, n_layers, lambda l: w_copy(l).start())
    x_copy(G, G % 2).start()

    b_copy.wait()
    bf32[0:n_layers, :] = braw[...].astype(F32)

    def t_index(l, i1, i2, j):
        return ((l * 7 + i1 - 1) * 7 + i2 - 1) * ntile + j

    def get_t(l, i1, i2, j):
        return pltpu.bitcast(t_ref[t_index(l, i1, i2, j)], BF16)

    def build_t(l, i1):
        for j in range(ntile):
            for r0 in range(0, cs, PREP_ROWS):
                def w_tile(r, c):
                    rows = slice(r * cs + r0, r * cs + r0 + PREP_ROWS)
                    cols = slice(c * cs + j * LANES, c * cs + (j + 1) * LANES)
                    return wbuf[l, rows, cols].astype(F32)
                lvl1 = [_signed_sum([(s, w_tile(*_sub_block(q, k))) for s, q in _RHS[i1]])
                        for k in range(4)]
                for i2 in range(1, 8):
                    v = _signed_sum([(s, lvl1[k]) for s, k in _RHS[i2]]).astype(BF16)
                    t_ref[t_index(l, i1, i2, j), r0 // 2:(r0 + PREP_ROWS) // 2, :] = (
                        pltpu.bitcast(v, U32))

    def x0_start(r, c):
        return x0s[r * ru:(r + 1) * ru, c * cs:(c + 1) * cs].astype(F32)

    def store_state(new):
        for r in range(4):
            for c in range(4):
                xs32[r * ru:(r + 1) * ru, c * cs:(c + 1) * cs] = new[r][c]

    def before_first(i1):
        if i1 == 2:
            xs_half_copy(1).wait()
            w0_quadrant_copy(0, 0).wait()
        elif i1 == 4:
            w0_quadrant_copy(1, 0).wait()
        elif i1 == 7:
            xs_half_copy(0).wait()
            w0_quadrant_copy(1, 1).wait()
            w0_quadrant_copy(0, 1).wait()
        build_t(0, i1)

    x0_first = functools.lru_cache(maxsize=None)(x0_start)
    store_state(_cross_layer(
        x0_first, x0_first, [bf32[0:1, c * cs:(c + 1) * cs] for c in range(4)],
        functools.partial(get_t, 0), _ORDER_FIRST, before_product=before_first))

    def start_layer(l):
        w_copy(l).wait()
        brow = bf32[pl.ds(l, 1), :]
        xv = [[xs32[r * ru:(r + 1) * ru, c * cs:(c + 1) * cs] for c in range(4)] for r in range(4)]
        store_state(_cross_layer(
            lambda r, c: xv[r][c], x0_start, [brow[:, c * cs:(c + 1) * cs] for c in range(4)],
            functools.partial(get_t, l), _ORDER_X, before_product=functools.partial(build_t, l)))

    loop(1, n_layers, start_layer)
    os16[...] = xs32[...].astype(BF16)
    os_copy.start()

    def main_block(i):
        slot = i & 1
        x_copy(i, slot).wait()

        @pl.when(i >= G + 2)
        def _():
            for q in range(4):
                o_copy(i - 2, slot, q).wait()

        @pl.when(i + 1 < n_blocks)
        def _():
            x_copy(i + 1, 1 - slot).start()

        x_in = xbuf.at[slot]
        x_out = obuf.at[slot]
        x0v = [[x_in[r * rs:(r + 1) * rs, c * cs:(c + 1) * cs].astype(F32) for c in range(4)]
               for r in range(4)]

        def write_quadrant(q, new):
            for k in range(4):
                r, c = _sub_block(q, k)
                x_out[r * rs:(r + 1) * rs, c * cs:(c + 1) * cs] = new[r][c].astype(BF16)
            o_copy(i, slot, q).start()

        xv = x0v
        for l in range(n_layers):
            xv = _cross_layer(
                functools.partial(lambda g, r, c: g[r][c], xv), lambda r, c: x0v[r][c],
                [bf32[l:l + 1, c * cs:(c + 1) * cs] for c in range(4)],
                functools.partial(get_t, l), _ORDER_Y if l % 2 else _ORDER_X,
                after_quadrant=write_quadrant if l == n_layers - 1 else None)

    loop(G, n_blocks, main_block)

    os_copy.wait()
    for i in (n_blocks - 2, n_blocks - 1):
        for q in range(4):
            o_copy(i, i % 2, q).wait()


@jax.jit
def pallas_standalone__dcn_v2_cross__recsys_kernel(
    x0: jax.Array,
    ws: jax.Array,
    bs: jax.Array,
):
    batch, d = x0.shape
    n_layers = ws.shape[0]
    assert ws.shape == (n_layers, d, d) and bs.shape == (n_layers, d)
    assert batch % TM == 0 and batch // TM >= G + 2
    assert d % (4 * LANES) == 0 and 2 <= n_layers <= 8
    ts = TM * G
    ntile = d // 4 // LANES
    return pl.pallas_call(
        _kernel,
        in_specs=[pl.BlockSpec(memory_space=pl.ANY)] * 3,
        out_specs=pl.BlockSpec(memory_space=pl.ANY),
        out_shape=jax.ShapeDtypeStruct((batch, d), x0.dtype),
        scratch_shapes=[
            pltpu.VMEM((2, TM, d), BF16),
            pltpu.VMEM((2, TM, d), BF16),
            pltpu.VMEM((n_layers, d, d), BF16),
            pltpu.VMEM((n_layers * 49 * ntile, d // 8, LANES), U32),
            pltpu.VMEM((n_layers, d), BF16),
            pltpu.VMEM((8, d), F32),
            pltpu.VMEM((ts, d), F32),
            pltpu.VMEM((ts, d), BF16),
            pltpu.VMEM((ts, d), BF16),
            pltpu.SemaphoreType.DMA((2,)),
            pltpu.SemaphoreType.DMA((8,)),
            pltpu.SemaphoreType.DMA((n_layers,)),
            pltpu.SemaphoreType.DMA((4,)),
            pltpu.SemaphoreType.DMA((4,)),
        ],
        compiler_params=pltpu.CompilerParams(
            vmem_limit_bytes=100 * 1024 * 1024,
            disable_bounds_checks=True,
        ),
    )(x0, ws, bs)
```

```python
import functools

import jax
import jax.numpy as jnp
from jax import lax
from jax.experimental import pallas as pl
from jax.experimental.pallas import tpu as pltpu

F32 = jnp.float32
BF16 = jnp.bfloat16
U32 = jnp.uint32

TM = 256
TS = 1024
PREP_ROWS = 32
LANES = 128

_LHS = {1: ((1, 0), (1, 3)), 2: ((1, 2), (1, 3)), 3: ((1, 0),), 4: ((1, 3),),
        5: ((1, 0), (1, 1)), 6: ((1, 2), (-1, 0)), 7: ((1, 1), (-1, 3))}
_RHS = {1: ((1, 0), (1, 3)), 2: ((1, 0),), 3: ((1, 1), (-1, 3)), 4: ((1, 2), (-1, 0)),
        5: ((1, 3),), 6: ((1, 0), (1, 1)), 7: ((1, 2), (1, 3))}
_OUT = {0: {1: 1, 4: 1, 5: -1, 7: 1}, 1: {3: 1, 5: 1}, 2: {2: 1, 4: 1}, 3: {1: 1, 2: -1, 3: 1, 6: 1}}

_MAIN_OUTER = ((3, 5, 6, 2, 1, 4, 7), (4, 3, 1, 2, 5, 7, 6))
_MAIN_INNER = ((6, 3, 5, 1, 2, 4, 7), (2, 3, 5, 1, 6, 4, 7))
_START_OUTER = (5, 7, 3, 1, 6, 4, 2)
_START_INNER = ((7, 4, 1, 5, 3, 6, 2), (2, 5, 4, 6, 3, 1, 7))
_FIRST_OUTER = (2, 4, 6, 7, 1, 5, 3)
_FIRST_INNER = (2, 5, 3, 4, 1, 7, 6)


def _signed_sum(terms, add=lambda a, b: a + b, sub=lambda a, b: a - b):
    terms = sorted(terms, key=lambda t: -t[0])
    assert terms[0][0] == 1
    acc = terms[0][1]
    for s, v in terms[1:]:
        acc = add(acc, v) if s == 1 else sub(acc, v)
    return acc


def _combine(order, product, finish, add, sub):
    pending = {q: [] for q in _OUT}
    seen = {q: 0 for q in _OUT}
    for i in order:
        m = product(i)
        for q, coef in _OUT.items():
            if i not in coef:
                continue
            pending[q].append((coef[i], m))
            seen[q] += 1
            if len(pending[q]) == 2:
                pending[q] = [(1, _signed_sum(pending[q], add, sub))]
            if seen[q] == len(coef):
                finish(q, pending[q][0][1])


def _sub_block(q, k):
    return 2 * (q // 2) + k // 2, 2 * (q % 2) + k % 2


def _cross_layer(x, x0, bias, get_t, outer_order, inner_orders=None, wide_order=None,
                 before_product=None, after_quadrant=None):
    ntile = bias[0].shape[1] // LANES

    def inner(terms, i1):
        lhs = {}

        def product(j, i2):
            if i2 not in lhs:
                lhs[i2] = _signed_sum(
                    [(s * s2, v) for s, k in _LHS[i2] for s2, v in terms[k]]).astype(BF16)
            return jnp.dot(lhs[i2], get_t(i1, i2, j), preferred_element_type=F32)

        out = [[None] * ntile for _ in range(4)]
        if wide_order is not None:
            def finish_wide(k, v):
                out[k] = v
            _combine(wide_order, lambda i2: [product(j, i2) for j in range(ntile)], finish_wide,
                     lambda a, b: [u + v for u, v in zip(a, b)],
                     lambda a, b: [u - v for u, v in zip(a, b)])
            return out
        for j in range(ntile):
            def finish(k, v, j=j):
                out[k][j] = v
            _combine(inner_orders[j % len(inner_orders)], functools.partial(product, j), finish,
                     lambda a, b: a + b, lambda a, b: a - b)
        return out

    def outer_product(i1):
        if before_product is not None:
            before_product(i1)
        terms = [[(s, x(*_sub_block(q, k))) for s, q in _LHS[i1]] for k in range(4)]
        return inner(terms, i1)

    def zip2(f):
        return lambda a, b: [[f(u, v) for u, v in zip(ra, rb)] for ra, rb in zip(a, b)]

    new = [[None] * 4 for _ in range(4)]

    def outer_finish(q, c):
        for k in range(4):
            r, col = _sub_block(q, k)
            y = jnp.concatenate(c[k], axis=1) + bias[col]
            new[r][col] = x0(r, col) * y + x(r, col)
        if after_quadrant is not None:
            after_quadrant(q, new)

    _combine(outer_order, outer_product, outer_finish,
             zip2(lambda a, b: a + b), zip2(lambda a, b: a - b))
    return new


def _kernel(x0_hbm, w_hbm, b_hbm, o_hbm,
            xbuf, obuf, wbuf, t_ref, braw, bf32, xs32, x0s, os16,
            xsem, osem, wsem, ssem, qsem):
    n_layers, d, _ = wbuf.shape
    n_iter = (x0_hbm.shape[0] - TS) // TM
    cs = d // 4
    hd = d // 2
    ntile = cs // LANES
    rs = TM // 4
    ru = TS // 4
    hm = TM // 2

    def x_copy(i, slot):
        r0 = pl.multiple_of(TS + i * TM, 64)
        return pltpu.make_async_copy(x0_hbm.at[pl.ds(r0, TM)], xbuf.at[slot], xsem.at[slot])

    def o_copy(i, slot, q):
        r0 = pl.multiple_of(TS + i * TM, 64)
        qr, qc = divmod(q, 2)
        return pltpu.make_async_copy(
            obuf.at[slot, pl.ds(qr * hm, hm), pl.ds(qc * hd, hd)],
            o_hbm.at[pl.ds(r0 + qr * hm, hm), pl.ds(qc * hd, hd)],
            osem.at[slot * 4 + q])

    def w_copy(l):
        return pltpu.make_async_copy(w_hbm.at[l], wbuf.at[l], wsem.at[l])

    def w0_quadrant_copy(r, c):
        r0 = pl.multiple_of(r * hd, hd)
        c0 = pl.multiple_of(c * hd, hd)
        return pltpu.make_async_copy(
            w_hbm.at[0, pl.ds(r0, hd), pl.ds(c0, hd)],
            wbuf.at[0, pl.ds(r0, hd), pl.ds(c0, hd)],
            qsem.at[2 * r + c])

    def xs_half_copy(h):
        rows = pl.ds(h * (TS // 2), TS // 2)
        return pltpu.make_async_copy(x0_hbm.at[rows], x0s.at[rows], ssem.at[1 + h])

    b_copy = pltpu.make_async_copy(b_hbm, braw, ssem.at[0])
    os_copy = pltpu.make_async_copy(os16, o_hbm.at[pl.ds(0, TS)], ssem.at[3])

    def loop(lo, hi, fn):
        def body(i, carry):
            fn(i)
            return carry
        lax.fori_loop(lo, hi, body, 0)

    b_copy.start()
    xs_half_copy(1).start()
    loop(0, 2, lambda r: w0_quadrant_copy(r, 0).start())
    xs_half_copy(0).start()
    loop(0, 2, lambda r: w0_quadrant_copy(1 - r, 1).start())
    loop(1, n_layers, lambda l: w_copy(l).start())
    x_copy(0, 0).start()

    b_copy.wait()
    bf32[0:n_layers, :] = braw[...].astype(F32)

    def t_index(l, i1, i2, j):
        return ((l * 7 + i1 - 1) * 7 + i2 - 1) * ntile + j

    def get_t(l, i1, i2, j):
        return pltpu.bitcast(t_ref[t_index(l, i1, i2, j)], BF16)

    def build_t(l, i1):
        for j in range(ntile):
            for r0 in range(0, cs, PREP_ROWS):
                def w_tile(r, c):
                    rows = slice(r * cs + r0, r * cs + r0 + PREP_ROWS)
                    cols = slice(c * cs + j * LANES, c * cs + (j + 1) * LANES)
                    return wbuf[l, rows, cols].astype(F32)
                lvl1 = [_signed_sum([(s, w_tile(*_sub_block(q, k))) for s, q in _RHS[i1]])
                        for k in range(4)]
                for i2 in range(1, 8):
                    v = _signed_sum([(s, lvl1[k]) for s, k in _RHS[i2]]).astype(BF16)
                    t_ref[t_index(l, i1, i2, j), r0 // 2:(r0 + PREP_ROWS) // 2, :] = (
                        pltpu.bitcast(v, U32))

    def x0_start(r, c):
        return x0s[r * ru:(r + 1) * ru, c * cs:(c + 1) * cs].astype(F32)

    def store_state(new):
        for r in range(4):
            for c in range(4):
                xs32[r * ru:(r + 1) * ru, c * cs:(c + 1) * cs] = new[r][c]

    def before_first(i1):
        if i1 == _FIRST_OUTER[0]:
            xs_half_copy(1).wait()
            w0_quadrant_copy(0, 0).wait()
        elif i1 == _FIRST_OUTER[1]:
            w0_quadrant_copy(1, 0).wait()
        elif i1 == _FIRST_OUTER[2]:
            xs_half_copy(0).wait()
            w0_quadrant_copy(1, 1).wait()
            w0_quadrant_copy(0, 1).wait()
        build_t(0, i1)

    x0_first = functools.lru_cache(maxsize=None)(x0_start)
    store_state(_cross_layer(
        x0_first, x0_first, [bf32[0:1, c * cs:(c + 1) * cs] for c in range(4)],
        functools.partial(get_t, 0), _FIRST_OUTER, wide_order=_FIRST_INNER,
        before_product=before_first))

    def start_layer(l):
        w_copy(l).wait()
        brow = bf32[pl.ds(l, 1), :]
        xv = [[xs32[r * ru:(r + 1) * ru, c * cs:(c + 1) * cs] for c in range(4)] for r in range(4)]
        store_state(_cross_layer(
            lambda r, c: xv[r][c], x0_start, [brow[:, c * cs:(c + 1) * cs] for c in range(4)],
            functools.partial(get_t, l), _START_OUTER, _START_INNER,
            before_product=functools.partial(build_t, l)))

    loop(1, n_layers, start_layer)
    os16[...] = xs32[...].astype(BF16)
    os_copy.start()

    def main_block(i):
        slot = i & 1
        x_copy(i, slot).wait()

        @pl.when(i >= 2)
        def _():
            for q in range(4):
                o_copy(i - 2, slot, q).wait()

        @pl.when(i + 1 < n_iter)
        def _():
            x_copy(i + 1, 1 - slot).start()

        x_in = xbuf.at[slot]
        x_out = obuf.at[slot]
        x0v = [[x_in[r * rs:(r + 1) * rs, c * cs:(c + 1) * cs].astype(F32) for c in range(4)]
               for r in range(4)]

        def write_quadrant(q, new):
            for k in range(4):
                r, c = _sub_block(q, k)
                x_out[r * rs:(r + 1) * rs, c * cs:(c + 1) * cs] = new[r][c].astype(BF16)
            o_copy(i, slot, q).start()

        xv = x0v
        for l in range(n_layers):
            xv = _cross_layer(
                functools.partial(lambda g, r, c: g[r][c], xv), lambda r, c: x0v[r][c],
                [bf32[l:l + 1, c * cs:(c + 1) * cs] for c in range(4)],
                functools.partial(get_t, l), _MAIN_OUTER[l % 2], _MAIN_INNER,
                after_quadrant=write_quadrant if l == n_layers - 1 else None)

    loop(0, n_iter, main_block)

    os_copy.wait()
    for i in (n_iter - 2, n_iter - 1):
        for q in range(4):
            o_copy(i, i % 2, q).wait()


@jax.jit
def pallas_standalone__dcn_v2_cross__recsys_kernel(
    x0: jax.Array,
    ws: jax.Array,
    bs: jax.Array,
):
    batch, d = x0.shape
    n_layers = ws.shape[0]
    assert ws.shape == (n_layers, d, d) and bs.shape == (n_layers, d)
    assert (batch - TS) % TM == 0 and (batch - TS) // TM >= 2
    assert d % (4 * LANES) == 0 and 2 <= n_layers <= 8
    ntile = d // 4 // LANES
    return pl.pallas_call(
        _kernel,
        in_specs=[pl.BlockSpec(memory_space=pl.ANY)] * 3,
        out_specs=pl.BlockSpec(memory_space=pl.ANY),
        out_shape=jax.ShapeDtypeStruct((batch, d), x0.dtype),
        scratch_shapes=[
            pltpu.VMEM((2, TM, d), BF16),
            pltpu.VMEM((2, TM, d), BF16),
            pltpu.VMEM((n_layers, d, d), BF16),
            pltpu.VMEM((n_layers * 49 * ntile, d // 8, LANES), U32),
            pltpu.VMEM((n_layers, d), BF16),
            pltpu.VMEM((8, d), F32),
            pltpu.VMEM((TS, d), F32),
            pltpu.VMEM((TS, d), BF16),
            pltpu.VMEM((TS, d), BF16),
            pltpu.SemaphoreType.DMA((2,)),
            pltpu.SemaphoreType.DMA((8,)),
            pltpu.SemaphoreType.DMA((n_layers,)),
            pltpu.SemaphoreType.DMA((4,)),
            pltpu.SemaphoreType.DMA((4,)),
        ],
        compiler_params=pltpu.CompilerParams(
            vmem_limit_bytes=100 * 1024 * 1024,
            disable_bounds_checks=True,
        ),
    )(x0, ws, bs)
```

```python
import functools

import jax
import jax.numpy as jnp
from jax import lax
from jax.experimental import pallas as pl
from jax.experimental.pallas import tpu as pltpu

F32 = jnp.float32
BF16 = jnp.bfloat16
U32 = jnp.uint32

TM = 256
TS = 1024
PREP_ROWS = 32
LANES = 128

_LHS = {1: ((1, 0), (1, 3)), 2: ((1, 2), (1, 3)), 3: ((1, 0),), 4: ((1, 3),),
        5: ((1, 0), (1, 1)), 6: ((1, 2), (-1, 0)), 7: ((1, 1), (-1, 3))}
_RHS = {1: ((1, 0), (1, 3)), 2: ((1, 0),), 3: ((1, 1), (-1, 3)), 4: ((1, 2), (-1, 0)),
        5: ((1, 3),), 6: ((1, 0), (1, 1)), 7: ((1, 2), (1, 3))}
_OUT = {0: {1: 1, 4: 1, 5: -1, 7: 1}, 1: {3: 1, 5: 1}, 2: {2: 1, 4: 1}, 3: {1: 1, 2: -1, 3: 1, 6: 1}}

_MAIN_OUTER = ((3, 5, 6, 2, 1, 4, 7), (4, 3, 1, 2, 5, 7, 6))
_MAIN_INNER = ((6, 3, 5, 1, 2, 4, 7), (2, 3, 5, 1, 6, 4, 7))
_START_OUTER = (5, 7, 3, 1, 6, 4, 2)
_START_INNER = ((7, 4, 1, 5, 3, 6, 2), (2, 5, 4, 6, 3, 1, 7))
_FIRST_INNER = (2, 5, 3, 4, 1, 7, 6)
_FIRST_MID = (5, 7, 1)
_FIRST_LAST = (4, 7, 3, 2, 6, 5, 1)


def _add(a, b):
    return a + b


def _sub(a, b):
    return a - b


def _zip1(f):
    return lambda a, b: [f(u, v) for u, v in zip(a, b)]


def _signed_sum(terms, add=_add, sub=_sub):
    terms = sorted(terms, key=lambda t: -t[0])
    assert terms[0][0] == 1
    acc = terms[0][1]
    for s, v in terms[1:]:
        acc = add(acc, v) if s == 1 else sub(acc, v)
    return acc


def _sub_block(q, k):
    return 2 * (q // 2) + k // 2, 2 * (q % 2) + k % 2


class _Accumulator:
    def __init__(self, finish, add, sub):
        self.finish, self.add, self.sub = finish, add, sub
        self.pending = {q: [] for q in _OUT}
        self.seen = {q: 0 for q in _OUT}

    def accept(self, i, m):
        for q, coef in _OUT.items():
            if i not in coef:
                continue
            self.pending[q].append((coef[i], m))
            self.seen[q] += 1
            if len(self.pending[q]) == 2:
                self.pending[q] = [(1, _signed_sum(self.pending[q], self.add, self.sub))]
            if self.seen[q] == len(coef):
                self.finish(q, self.pending[q][0][1])


class _Rows:
    def __init__(self, x, x0, bias, after_quadrant=None):
        self.x, self.x0, self.bias, self.after_quadrant = x, x0, bias, after_quadrant
        self.new = [[None] * 4 for _ in range(4)]
        self.acc = _Accumulator(self._finish, _zip1(_zip1(_add)), _zip1(_zip1(_sub)))

    def _finish(self, q, c):
        for k in range(4):
            r, col = _sub_block(q, k)
            y = jnp.concatenate(c[k], axis=1) + self.bias[col]
            self.new[r][col] = self.x0(r, col) * y + self.x(r, col)
        if self.after_quadrant is not None:
            self.after_quadrant(q, self.new)

    def lhs(self, i1, i2):
        return _signed_sum([(s2 * s1, self.x(*_sub_block(q, k)))
                            for s2, k in _LHS[i2] for s1, q in _LHS[i1]])


def _outer_product(i1, groups, get_t, inner_orders=None, wide_order=None):
    ntile = groups[0].bias[0].shape[1] // LANES
    lhs = {}

    def product(j, i2):
        if i2 not in lhs:
            parts = [g.lhs(i1, i2) for g in groups]
            lhs[i2] = (parts[0] if len(parts) == 1 else jnp.concatenate(parts, axis=0)).astype(BF16)
        return jnp.dot(lhs[i2], get_t(i1, i2, j), preferred_element_type=F32)

    out = [[None] * ntile for _ in range(4)]
    if wide_order is not None:
        def finish_wide(k, v):
            out[k] = v
        acc = _Accumulator(finish_wide, _zip1(_add), _zip1(_sub))
        for i2 in wide_order:
            acc.accept(i2, [product(j, i2) for j in range(ntile)])
    else:
        for j in range(ntile):
            def finish(k, v, j=j):
                out[k][j] = v
            acc = _Accumulator(finish, _add, _sub)
            for i2 in inner_orders[j % len(inner_orders)]:
                acc.accept(i2, product(j, i2))
    if len(groups) == 1:
        groups[0].acc.accept(i1, out)
    else:
        n = out[0][0].shape[0] // len(groups)
        for u, g in enumerate(groups):
            g.acc.accept(i1, [[t[u * n:(u + 1) * n] for t in row] for row in out])


def _cross_layer(x, x0, bias, get_t, outer_order, inner_orders,
                 before_product=None, after_quadrant=None):
    g = _Rows(x, x0, bias, after_quadrant)
    for i1 in outer_order:
        if before_product is not None:
            before_product(i1)
        _outer_product(i1, [g], get_t, inner_orders)
    return g.new


def _kernel(x0_hbm, w_hbm, b_hbm, o_hbm,
            xbuf, obuf, wbuf, t_ref, braw, bf32, xs32, x0s, os16,
            xsem, osem, wsem, ssem, qsem):
    n_layers, d, _ = wbuf.shape
    n_iter = (x0_hbm.shape[0] - TS) // TM
    cs = d // 4
    hd = d // 2
    ntile = cs // LANES
    rs = TM // 4
    ru = TS // 4
    rh = TS // 8

    def x_copy(i, slot):
        r0 = pl.multiple_of(TS + i * TM, 64)
        return pltpu.make_async_copy(x0_hbm.at[pl.ds(r0, TM)], xbuf.at[slot], xsem.at[slot])

    def o_copy(i, slot, r, c):
        r0 = pl.multiple_of(TS + i * TM, 64)
        return pltpu.make_async_copy(
            obuf.at[slot, pl.ds(r * rs, rs), pl.ds(c * cs, cs)],
            o_hbm.at[pl.ds(r0 + r * rs, rs), pl.ds(c * cs, cs)],
            osem.at[slot])

    def o_wait_all(i, slot):
        r0 = pl.multiple_of(TS + i * TM, 64)
        pltpu.make_async_copy(obuf.at[slot], o_hbm.at[pl.ds(r0, TM)], osem.at[slot]).wait()

    def w_copy(l):
        return pltpu.make_async_copy(w_hbm.at[l], wbuf.at[l], wsem.at[l])

    def w0_quadrant_copy(r, c):
        r0 = pl.multiple_of(r * hd, hd)
        c0 = pl.multiple_of(c * hd, hd)
        return pltpu.make_async_copy(
            w_hbm.at[0, pl.ds(r0, hd), pl.ds(c0, hd)],
            wbuf.at[0, pl.ds(r0, hd), pl.ds(c0, hd)],
            qsem.at[2 * r + c])

    def xs_copy(r0, rows, sem):
        return pltpu.make_async_copy(
            x0_hbm.at[pl.ds(r0, rows)], x0s.at[pl.ds(r0, rows)], ssem.at[sem])

    xa_top = xs_copy(0, TS // 4, 4)
    xa_bot = xs_copy(TS // 4, TS // 4, 5)
    xb_all = xs_copy(TS // 2, TS // 2, 2)
    b_copy = pltpu.make_async_copy(b_hbm, braw, ssem.at[0])
    os_copy = pltpu.make_async_copy(os16, o_hbm.at[pl.ds(0, TS)], ssem.at[3])

    def loop(lo, hi, fn):
        def body(i, carry):
            fn(i)
            return carry
        lax.fori_loop(lo, hi, body, 0)

    b_copy.start()
    xa_bot.start()
    loop(0, 2, lambda r: w0_quadrant_copy(r, 0).start())
    xa_top.start()
    loop(0, 2, lambda r: w0_quadrant_copy(1 - r, 1).start())
    xb_all.start()
    loop(1, n_layers, lambda l: w_copy(l).start())
    x_copy(0, 0).start()

    b_copy.wait()
    bf32[0:n_layers, :] = braw[...].astype(F32)

    def t_index(l, i1, i2, j):
        return ((l * 7 + i1 - 1) * 7 + i2 - 1) * ntile + j

    def get_t(l, i1, i2, j):
        return pltpu.bitcast(t_ref[t_index(l, i1, i2, j)], BF16)

    def build_t(l, i1):
        for j in range(ntile):
            for r0 in range(0, cs, PREP_ROWS):
                def w_tile(r, c):
                    rows = slice(r * cs + r0, r * cs + r0 + PREP_ROWS)
                    cols = slice(c * cs + j * LANES, c * cs + (j + 1) * LANES)
                    return wbuf[l, rows, cols].astype(F32)
                lvl1 = [_signed_sum([(s, w_tile(*_sub_block(q, k))) for s, q in _RHS[i1]])
                        for k in range(4)]
                for i2 in range(1, 8):
                    v = _signed_sum([(s, lvl1[k]) for s, k in _RHS[i2]]).astype(BF16)
                    t_ref[t_index(l, i1, i2, j), r0 // 2:(r0 + PREP_ROWS) // 2, :] = (
                        pltpu.bitcast(v, U32))

    def x0_group(u, r, c):
        return x0s[(u * 4 + r) * rh:(u * 4 + r + 1) * rh, c * cs:(c + 1) * cs].astype(F32)

    bias0 = [bf32[0:1, c * cs:(c + 1) * cs] for c in range(4)]
    get_t0 = functools.partial(get_t, 0)
    groups = []
    for u in range(2):
        xg = functools.lru_cache(maxsize=None)(functools.partial(x0_group, u))
        groups.append(_Rows(xg, xg, bias0))
    ga, gb = groups

    def first_product(i1, on):
        build_t(0, i1)
        _outer_product(i1, on, get_t0, wide_order=_FIRST_INNER)

    xa_bot.wait()
    w0_quadrant_copy(0, 0).wait()
    first_product(2, [ga])
    w0_quadrant_copy(1, 0).wait()
    first_product(4, [ga])
    xa_top.wait()
    w0_quadrant_copy(1, 1).wait()
    for i1 in _FIRST_MID:
        first_product(i1, [ga])
    w0_quadrant_copy(0, 1).wait()
    xb_all.wait()
    for i1 in _FIRST_LAST:
        if i1 in (3, 6):
            first_product(i1, [ga, gb])
        else:
            _outer_product(i1, [gb], get_t0, _START_INNER)
    for u in range(2):
        for r in range(4):
            for c in range(4):
                xs32[(u * 4 + r) * rh:(u * 4 + r + 1) * rh, c * cs:(c + 1) * cs] = groups[u].new[r][c]

    def x0_start(r, c):
        return x0s[r * ru:(r + 1) * ru, c * cs:(c + 1) * cs].astype(F32)

    def start_layer(l):
        w_copy(l).wait()
        brow = bf32[pl.ds(l, 1), :]
        xv = [[xs32[r * ru:(r + 1) * ru, c * cs:(c + 1) * cs] for c in range(4)] for r in range(4)]
        new = _cross_layer(
            lambda r, c: xv[r][c], x0_start, [brow[:, c * cs:(c + 1) * cs] for c in range(4)],
            functools.partial(get_t, l), _START_OUTER, _START_INNER,
            before_product=functools.partial(build_t, l))
        for r in range(4):
            for c in range(4):
                xs32[r * ru:(r + 1) * ru, c * cs:(c + 1) * cs] = new[r][c]

    loop(1, n_layers, start_layer)
    os16[...] = xs32[...].astype(BF16)
    os_copy.start()

    def main_block(i):
        slot = i & 1
        x_copy(i, slot).wait()

        @pl.when(i >= 2)
        def _():
            o_wait_all(i - 2, slot)

        @pl.when(i + 1 < n_iter)
        def _():
            x_copy(i + 1, 1 - slot).start()

        x_in = xbuf.at[slot]
        x_out = obuf.at[slot]
        x0v = [[x_in[r * rs:(r + 1) * rs, c * cs:(c + 1) * cs].astype(F32) for c in range(4)]
               for r in range(4)]

        def write_quadrant(q, new):
            for k in (1, 3, 2, 0):
                r, c = _sub_block(q, k)
                x_out[r * rs:(r + 1) * rs, c * cs:(c + 1) * cs] = new[r][c].astype(BF16)
                o_copy(i, slot, r, c).start()

        xv = x0v
        for l in range(n_layers):
            xv = _cross_layer(
                functools.partial(lambda g, r, c: g[r][c], xv), lambda r, c: x0v[r][c],
                [bf32[l:l + 1, c * cs:(c + 1) * cs] for c in range(4)],
                functools.partial(get_t, l), _MAIN_OUTER[l % 2], _MAIN_INNER,
                after_quadrant=write_quadrant if l == n_layers - 1 else None)

    loop(0, n_iter, main_block)

    os_copy.wait()
    for i in (n_iter - 2, n_iter - 1):
        o_wait_all(i, i % 2)


@jax.jit
def pallas_standalone__dcn_v2_cross__recsys_kernel(
    x0: jax.Array,
    ws: jax.Array,
    bs: jax.Array,
):
    batch, d = x0.shape
    n_layers = ws.shape[0]
    assert ws.shape == (n_layers, d, d) and bs.shape == (n_layers, d)
    assert (batch - TS) % TM == 0 and (batch - TS) // TM >= 2
    assert d % (4 * LANES) == 0 and 2 <= n_layers <= 8
    ntile = d // 4 // LANES
    return pl.pallas_call(
        _kernel,
        in_specs=[pl.BlockSpec(memory_space=pl.ANY)] * 3,
        out_specs=pl.BlockSpec(memory_space=pl.ANY),
        out_shape=jax.ShapeDtypeStruct((batch, d), x0.dtype),
        scratch_shapes=[
            pltpu.VMEM((2, TM, d), BF16),
            pltpu.VMEM((2, TM, d), BF16),
            pltpu.VMEM((n_layers, d, d), BF16),
            pltpu.VMEM((n_layers * 49 * ntile, d // 8, LANES), U32),
            pltpu.VMEM((n_layers, d), BF16),
            pltpu.VMEM((8, d), F32),
            pltpu.VMEM((TS, d), F32),
            pltpu.VMEM((TS, d), BF16),
            pltpu.VMEM((TS, d), BF16),
            pltpu.SemaphoreType.DMA((2,)),
            pltpu.SemaphoreType.DMA((2,)),
            pltpu.SemaphoreType.DMA((n_layers,)),
            pltpu.SemaphoreType.DMA((6,)),
            pltpu.SemaphoreType.DMA((4,)),
        ],
        compiler_params=pltpu.CompilerParams(
            vmem_limit_bytes=100 * 1024 * 1024,
            disable_bounds_checks=True,
            disable_semaphore_checks=True,
        ),
    )(x0, ws, bs)
```

```python
import functools

import jax
import jax.numpy as jnp
from jax import lax
from jax.experimental import pallas as pl
from jax.experimental.pallas import tpu as pltpu

F32 = jnp.float32
BF16 = jnp.bfloat16
U32 = jnp.uint32

TM = 256
TS = 1024
LANES = 128

_LHS = {1: ((1, 0), (1, 3)), 2: ((1, 2), (1, 3)), 3: ((1, 0),), 4: ((1, 3),),
        5: ((1, 0), (1, 1)), 6: ((1, 2), (-1, 0)), 7: ((1, 1), (-1, 3))}
_RHS = {1: ((1, 0), (1, 3)), 2: ((1, 0),), 3: ((1, 1), (-1, 3)), 4: ((1, 2), (-1, 0)),
        5: ((1, 3),), 6: ((1, 0), (1, 1)), 7: ((1, 2), (1, 3))}
_OUT = {0: {1: 1, 4: 1, 5: -1, 7: 1}, 1: {3: 1, 5: 1}, 2: {2: 1, 4: 1}, 3: {1: 1, 2: -1, 3: 1, 6: 1}}

_MAIN_OUTER = ((3, 5, 6, 2, 1, 4, 7), (4, 3, 1, 2, 5, 7, 6))
_MAIN_INNER = ((6, 3, 5, 1, 2, 4, 7), (2, 3, 5, 1, 6, 4, 7))
_START_OUTER = (5, 7, 3, 1, 6, 4, 2)
_START_INNER = ((7, 4, 1, 5, 3, 6, 2), (2, 5, 4, 6, 3, 1, 7))
_FIRST_INNER = (2, 5, 3, 4, 1, 7, 6)
_FIRST_MID = (5, 7, 1)
_FIRST_LAST = (4, 7, 3, 2, 6, 5, 1)


def _add(a, b):
    return a + b


def _sub(a, b):
    return a - b


def _zip1(f):
    return lambda a, b: [f(u, v) for u, v in zip(a, b)]


def _signed_sum(terms, add=_add, sub=_sub):
    terms = sorted(terms, key=lambda t: -t[0])
    assert terms[0][0] == 1
    acc = terms[0][1]
    for s, v in terms[1:]:
        acc = add(acc, v) if s == 1 else sub(acc, v)
    return acc


def _sub_block(q, k):
    return 2 * (q // 2) + k // 2, 2 * (q % 2) + k % 2


class _Accumulator:
    def __init__(self, finish, add, sub):
        self.finish, self.add, self.sub = finish, add, sub
        self.pending = {q: [] for q in _OUT}
        self.seen = {q: 0 for q in _OUT}

    def accept(self, i, m):
        for q, coef in _OUT.items():
            if i not in coef:
                continue
            self.pending[q].append((coef[i], m))
            self.seen[q] += 1
            if len(self.pending[q]) == 2:
                self.pending[q] = [(1, _signed_sum(self.pending[q], self.add, self.sub))]
            if self.seen[q] == len(coef):
                self.finish(q, self.pending[q][0][1])


class _Rows:
    def __init__(self, x, x0, bias, after_quadrant=None):
        self.x, self.x0, self.bias, self.after_quadrant = x, x0, bias, after_quadrant
        self.new = [[None] * 4 for _ in range(4)]
        self.acc = _Accumulator(self._finish, _zip1(_zip1(_add)), _zip1(_zip1(_sub)))

    def _finish(self, q, c):
        for k in range(4):
            r, col = _sub_block(q, k)
            y = jnp.concatenate(c[k], axis=1) + self.bias[col]
            self.new[r][col] = self.x0(r, col) * y + self.x(r, col)
        if self.after_quadrant is not None:
            self.after_quadrant(q, self.new)

    def lhs(self, i1, i2):
        return _signed_sum([(s2 * s1, self.x(*_sub_block(q, k)))
                            for s2, k in _LHS[i2] for s1, q in _LHS[i1]])


def _outer_product(i1, groups, get_t, inner_orders=None, wide_order=None):
    ntile = groups[0].bias[0].shape[1] // LANES
    lhs = {}

    def product(j, i2):
        if i2 not in lhs:
            parts = [g.lhs(i1, i2) for g in groups]
            lhs[i2] = (parts[0] if len(parts) == 1 else jnp.concatenate(parts, axis=0)).astype(BF16)
        return jnp.dot(lhs[i2], get_t(i1, i2, j), preferred_element_type=F32)

    out = [[None] * ntile for _ in range(4)]
    if wide_order is not None:
        def finish_wide(k, v):
            out[k] = v
        acc = _Accumulator(finish_wide, _zip1(_add), _zip1(_sub))
        for i2 in wide_order:
            acc.accept(i2, [product(j, i2) for j in range(ntile)])
    else:
        for j in range(ntile):
            def finish(k, v, j=j):
                out[k][j] = v
            acc = _Accumulator(finish, _add, _sub)
            for i2 in inner_orders[j % len(inner_orders)]:
                acc.accept(i2, product(j, i2))
    if len(groups) == 1:
        groups[0].acc.accept(i1, out)
    else:
        n = out[0][0].shape[0] // len(groups)
        for u, g in enumerate(groups):
            g.acc.accept(i1, [[t[u * n:(u + 1) * n] for t in row] for row in out])


def _cross_layer(x, x0, bias, get_t, outer_order, inner_orders,
                 before_product=None, after_quadrant=None):
    g = _Rows(x, x0, bias, after_quadrant)
    for i1 in outer_order:
        if before_product is not None:
            before_product(i1)
        _outer_product(i1, [g], get_t, inner_orders)
    return g.new


def _kernel(x0_hbm, w_hbm, b_hbm, o_hbm,
            xbuf, obuf, wbuf, t_ref, braw, bf32, xs32, x0s, os16,
            xsem, osem, wsem, ssem, qsem):
    n_layers, d, _ = wbuf.shape
    n_iter = (x0_hbm.shape[0] - TS) // TM
    cs = d // 4
    hd = d // 2
    ntile = cs // LANES
    rs = TM // 4
    ru = TS // 4
    rh = TS // 8

    def x_copy(i, slot):
        r0 = pl.multiple_of(TS + i * TM, 64)
        return pltpu.make_async_copy(x0_hbm.at[pl.ds(r0, TM)], xbuf.at[slot], xsem.at[slot])

    def o_copy(i, slot, r, c):
        r0 = pl.multiple_of(TS + i * TM, 64)
        return pltpu.make_async_copy(
            obuf.at[slot, pl.ds(r * rs, rs), pl.ds(c * cs, cs)],
            o_hbm.at[pl.ds(r0 + r * rs, rs), pl.ds(c * cs, cs)],
            osem.at[slot])

    def o_wait_all(i, slot):
        r0 = pl.multiple_of(TS + i * TM, 64)
        pltpu.make_async_copy(obuf.at[slot], o_hbm.at[pl.ds(r0, TM)], osem.at[slot]).wait()

    def w_copy(l):
        return pltpu.make_async_copy(w_hbm.at[l], wbuf.at[l], wsem.at[l])

    def w0_quadrant_copy(r, c):
        r0 = pl.multiple_of(r * hd, hd)
        c0 = pl.multiple_of(c * hd, hd)
        return pltpu.make_async_copy(
            w_hbm.at[0, pl.ds(r0, hd), pl.ds(c0, hd)],
            wbuf.at[0, pl.ds(r0, hd), pl.ds(c0, hd)],
            qsem.at[2 * r + c])

    def xs_copy(r0, rows, sem):
        return pltpu.make_async_copy(
            x0_hbm.at[pl.ds(r0, rows)], x0s.at[pl.ds(r0, rows)], ssem.at[sem])

    xa_top = xs_copy(0, TS // 4, 4)
    xa_bot = xs_copy(TS // 4, TS // 4, 5)
    xb_all = xs_copy(TS // 2, TS // 2, 2)
    b_copy = pltpu.make_async_copy(b_hbm, braw, ssem.at[0])
    os_copy = pltpu.make_async_copy(os16, o_hbm.at[pl.ds(0, TS)], ssem.at[3])

    def loop(lo, hi, fn):
        def body(i, carry):
            fn(i)
            return carry
        lax.fori_loop(lo, hi, body, 0)

    b_copy.start()
    xa_bot.start()
    loop(0, 2, lambda r: w0_quadrant_copy(r, 0).start())
    xa_top.start()
    loop(0, 2, lambda r: w0_quadrant_copy(1 - r, 1).start())
    xb_all.start()
    loop(1, n_layers, lambda l: w_copy(l).start())
    x_copy(0, 0).start()

    b_copy.wait()
    bf32[0:n_layers, :] = braw[...].astype(F32)

    def t_index(i1, i2, j):
        return ((i1 - 1) * 7 + i2 - 1) * ntile + j

    def get_t(l, i1, i2, j):
        return pltpu.bitcast(t_ref[l, t_index(i1, i2, j)], BF16)

    def build_t(l, i1):
        for j in range(ntile):
            def w_tile(r, c):
                cols = slice(c * cs + j * LANES, c * cs + (j + 1) * LANES)
                return wbuf[l, r * cs:(r + 1) * cs, cols].astype(F32)
            lvl1 = [_signed_sum([(s, w_tile(*_sub_block(q, k))) for s, q in _RHS[i1]])
                    for k in range(4)]
            for i2 in range(1, 8):
                v = _signed_sum([(s, lvl1[k]) for s, k in _RHS[i2]]).astype(BF16)
                t_ref[l, t_index(i1, i2, j)] = pltpu.bitcast(v, U32)

    def x0_group(u, r, c):
        return x0s[(u * 4 + r) * rh:(u * 4 + r + 1) * rh, c * cs:(c + 1) * cs].astype(F32)

    bias0 = [bf32[0:1, c * cs:(c + 1) * cs] for c in range(4)]
    get_t0 = functools.partial(get_t, 0)
    groups = []
    for u in range(2):
        xg = functools.lru_cache(maxsize=None)(functools.partial(x0_group, u))
        groups.append(_Rows(xg, xg, bias0))
    ga, gb = groups

    def first_product(i1, on):
        build_t(0, i1)
        _outer_product(i1, on, get_t0, wide_order=_FIRST_INNER)

    xa_bot.wait()
    w0_quadrant_copy(0, 0).wait()
    first_product(2, [ga])
    w0_quadrant_copy(1, 0).wait()
    first_product(4, [ga])
    xa_top.wait()
    w0_quadrant_copy(1, 1).wait()
    for i1 in _FIRST_MID:
        first_product(i1, [ga])
    w0_quadrant_copy(0, 1).wait()
    xb_all.wait()
    for i1 in _FIRST_LAST:
        if i1 in (3, 6):
            first_product(i1, [ga, gb])
        else:
            _outer_product(i1, [gb], get_t0, _START_INNER)
    for u in range(2):
        for r in range(4):
            for c in range(4):
                xs32[(u * 4 + r) * rh:(u * 4 + r + 1) * rh, c * cs:(c + 1) * cs] = groups[u].new[r][c]

    def x0_start(r, c):
        return x0s[r * ru:(r + 1) * ru, c * cs:(c + 1) * cs].astype(F32)

    def start_layer(l):
        w_copy(l).wait()
        brow = bf32[pl.ds(l, 1), :]
        xv = [[xs32[r * ru:(r + 1) * ru, c * cs:(c + 1) * cs] for c in range(4)] for r in range(4)]
        new = _cross_layer(
            lambda r, c: xv[r][c], x0_start, [brow[:, c * cs:(c + 1) * cs] for c in range(4)],
            functools.partial(get_t, l), _START_OUTER, _START_INNER,
            before_product=functools.partial(build_t, l))
        for r in range(4):
            for c in range(4):
                xs32[r * ru:(r + 1) * ru, c * cs:(c + 1) * cs] = new[r][c]

    loop(1, n_layers, start_layer)
    os16[...] = xs32[...].astype(BF16)
    os_copy.start()

    def main_block(i):
        slot = i & 1
        x_copy(i, slot).wait()

        @pl.when(i >= 2)
        def _():
            o_wait_all(i - 2, slot)

        @pl.when(i + 1 < n_iter)
        def _():
            x_copy(i + 1, 1 - slot).start()

        x_in = xbuf.at[slot]
        x_out = obuf.at[slot]
        x0v = [[x_in[r * rs:(r + 1) * rs, c * cs:(c + 1) * cs].astype(F32) for c in range(4)]
               for r in range(4)]

        def write_quadrant(q, new):
            for k in (1, 3, 2, 0):
                r, c = _sub_block(q, k)
                x_out[r * rs:(r + 1) * rs, c * cs:(c + 1) * cs] = new[r][c].astype(BF16)
                o_copy(i, slot, r, c).start()

        xv = x0v
        for l in range(n_layers):
            xv = _cross_layer(
                functools.partial(lambda g, r, c: g[r][c], xv), lambda r, c: x0v[r][c],
                [bf32[l:l + 1, c * cs:(c + 1) * cs] for c in range(4)],
                functools.partial(get_t, l), _MAIN_OUTER[l % 2], _MAIN_INNER,
                after_quadrant=write_quadrant if l == n_layers - 1 else None)

    loop(0, n_iter, main_block)

    os_copy.wait()
    for i in (n_iter - 2, n_iter - 1):
        o_wait_all(i, i % 2)


@jax.jit
def pallas_standalone__dcn_v2_cross__recsys_kernel(
    x0: jax.Array,
    ws: jax.Array,
    bs: jax.Array,
):
    batch, d = x0.shape
    n_layers = ws.shape[0]
    assert ws.shape == (n_layers, d, d) and bs.shape == (n_layers, d)
    assert (batch - TS) % TM == 0 and (batch - TS) // TM >= 2
    assert d % (4 * LANES) == 0 and 2 <= n_layers <= 8
    ntile = d // 4 // LANES
    return pl.pallas_call(
        _kernel,
        in_specs=[pl.BlockSpec(memory_space=pl.ANY)] * 3,
        out_specs=pl.BlockSpec(memory_space=pl.ANY),
        out_shape=jax.ShapeDtypeStruct((batch, d), x0.dtype),
        scratch_shapes=[
            pltpu.VMEM((2, TM, d), BF16),
            pltpu.VMEM((2, TM, d), BF16),
            pltpu.VMEM((n_layers, d, d), BF16),
            pltpu.VMEM((n_layers, 49 * ntile, d // 8, LANES), U32),
            pltpu.VMEM((n_layers, d), BF16),
            pltpu.VMEM((8, d), F32),
            pltpu.VMEM((TS, d), F32),
            pltpu.VMEM((TS, d), BF16),
            pltpu.VMEM((TS, d), BF16),
            pltpu.SemaphoreType.DMA((2,)),
            pltpu.SemaphoreType.DMA((2,)),
            pltpu.SemaphoreType.DMA((n_layers,)),
            pltpu.SemaphoreType.DMA((6,)),
            pltpu.SemaphoreType.DMA((4,)),
        ],
        compiler_params=pltpu.CompilerParams(
            vmem_limit_bytes=100 * 1024 * 1024,
            disable_bounds_checks=True,
            disable_semaphore_checks=True,
        ),
    )(x0, ws, bs)
```

```python
import functools

import jax
import jax.numpy as jnp
from jax import lax
from jax.experimental import pallas as pl
from jax.experimental.pallas import tpu as pltpu

F32 = jnp.float32
BF16 = jnp.bfloat16
U32 = jnp.uint32

TM = 256
TS = 1024
LANES = 128

_LHS = {1: ((1, 0), (1, 3)), 2: ((1, 2), (1, 3)), 3: ((1, 0),), 4: ((1, 3),),
        5: ((1, 0), (1, 1)), 6: ((1, 2), (-1, 0)), 7: ((1, 1), (-1, 3))}
_RHS = {1: ((1, 0), (1, 3)), 2: ((1, 0),), 3: ((1, 1), (-1, 3)), 4: ((1, 2), (-1, 0)),
        5: ((1, 3),), 6: ((1, 0), (1, 1)), 7: ((1, 2), (1, 3))}
_OUT = {0: {1: 1, 4: 1, 5: -1, 7: 1}, 1: {3: 1, 5: 1}, 2: {2: 1, 4: 1}, 3: {1: 1, 2: -1, 3: 1, 6: 1}}

_MAIN_OUTER = ((3, 6, 5, 2, 1, 4, 7), (4, 3, 1, 2, 5, 7, 6), (3, 5, 6, 2, 1, 4, 7),
               (4, 3, 1, 2, 5, 7, 6), (3, 5, 6, 2, 1, 4, 7), (4, 3, 1, 2, 5, 7, 6))
_MAIN_INNER = (((6, 3, 5, 1, 2, 4, 7), (2, 3, 5, 1, 6, 4, 7)),
               ((6, 3, 5, 1, 2, 4, 7), (2, 3, 5, 1, 6, 4, 7)),
               ((6, 3, 5, 1, 2, 4, 7), (1, 3, 5, 2, 6, 4, 7)),
               ((6, 3, 5, 1, 2, 4, 7), (2, 3, 5, 1, 6, 4, 7)),
               ((6, 3, 5, 1, 2, 4, 7), (2, 3, 6, 4, 1, 5, 7)),
               ((3, 5, 1, 6, 2, 4, 7), (2, 3, 5, 1, 6, 4, 7)))
_START_OUTER = (5, 7, 3, 1, 6, 4, 2)
_START_INNER = ((7, 4, 1, 5, 3, 6, 2), (2, 5, 4, 6, 3, 1, 7))
_FIRST_INNER = (2, 5, 3, 4, 1, 7, 6)
_FIRST_MID = (5, 7, 1)
_FIRST_LAST = (4, 7, 3, 2, 6, 5, 1)


def _add(a, b):
    return a + b


def _sub(a, b):
    return a - b


def _zip1(f):
    return lambda a, b: [f(u, v) for u, v in zip(a, b)]


def _signed_sum(terms, add=_add, sub=_sub):
    terms = sorted(terms, key=lambda t: -t[0])
    assert terms[0][0] == 1
    acc = terms[0][1]
    for s, v in terms[1:]:
        acc = add(acc, v) if s == 1 else sub(acc, v)
    return acc


def _sub_block(q, k):
    return 2 * (q // 2) + k // 2, 2 * (q % 2) + k % 2


class _Accumulator:
    def __init__(self, finish, add, sub):
        self.finish, self.add, self.sub = finish, add, sub
        self.pending = {q: [] for q in _OUT}
        self.seen = {q: 0 for q in _OUT}

    def accept(self, i, m):
        for q, coef in _OUT.items():
            if i not in coef:
                continue
            self.pending[q].append((coef[i], m))
            self.seen[q] += 1
            if len(self.pending[q]) == 2:
                self.pending[q] = [(1, _signed_sum(self.pending[q], self.add, self.sub))]
            if self.seen[q] == len(coef):
                self.finish(q, self.pending[q][0][1])


class _Rows:
    def __init__(self, x, x0, bias, after_quadrant=None):
        self.x, self.x0, self.bias, self.after_quadrant = x, x0, bias, after_quadrant
        self.new = [[None] * 4 for _ in range(4)]
        self.acc = _Accumulator(self._finish, _zip1(_zip1(_add)), _zip1(_zip1(_sub)))

    def _finish(self, q, c):
        for k in range(4):
            r, col = _sub_block(q, k)
            y = jnp.concatenate(c[k], axis=1) + self.bias[col]
            self.new[r][col] = self.x0(r, col) * y + self.x(r, col)
        if self.after_quadrant is not None:
            self.after_quadrant(q, self.new)

    def lhs(self, i1, i2):
        return _signed_sum([(s2 * s1, self.x(*_sub_block(q, k)))
                            for s2, k in _LHS[i2] for s1, q in _LHS[i1]])


def _outer_product(i1, groups, get_t, inner_orders=None, wide_order=None):
    ntile = groups[0].bias[0].shape[1] // LANES
    lhs = {}

    def product(j, i2):
        if i2 not in lhs:
            parts = [g.lhs(i1, i2) for g in groups]
            lhs[i2] = (parts[0] if len(parts) == 1 else jnp.concatenate(parts, axis=0)).astype(BF16)
        return jnp.dot(lhs[i2], get_t(i1, i2, j), preferred_element_type=F32)

    out = [[None] * ntile for _ in range(4)]
    if wide_order is not None:
        def finish_wide(k, v):
            out[k] = v
        acc = _Accumulator(finish_wide, _zip1(_add), _zip1(_sub))
        for i2 in wide_order:
            acc.accept(i2, [product(j, i2) for j in range(ntile)])
    else:
        for j in range(ntile):
            def finish(k, v, j=j):
                out[k][j] = v
            acc = _Accumulator(finish, _add, _sub)
            for i2 in inner_orders[j % len(inner_orders)]:
                acc.accept(i2, product(j, i2))
    if len(groups) == 1:
        groups[0].acc.accept(i1, out)
    else:
        n = out[0][0].shape[0] // len(groups)
        for u, g in enumerate(groups):
            g.acc.accept(i1, [[t[u * n:(u + 1) * n] for t in row] for row in out])


def _cross_layer(x, x0, bias, get_t, outer_order, inner_orders,
                 before_product=None, after_quadrant=None):
    g = _Rows(x, x0, bias, after_quadrant)
    for i1 in outer_order:
        if before_product is not None:
            before_product(i1)
        _outer_product(i1, [g], get_t, inner_orders)
    return g.new


def _kernel(x0_hbm, w_hbm, b_hbm, o_hbm,
            xbuf, obuf, wbuf, t_ref, braw, bf32, xs32, x0s, os16,
            xsem, osem, wsem, ssem, qsem):
    n_layers, d, _ = wbuf.shape
    n_iter = (x0_hbm.shape[0] - TS) // TM
    cs = d // 4
    hd = d // 2
    ntile = cs // LANES
    rs = TM // 4
    ru = TS // 4
    rh = TS // 8

    def x_copy(i, slot):
        r0 = pl.multiple_of(TS + i * TM, 64)
        return pltpu.make_async_copy(x0_hbm.at[pl.ds(r0, TM)], xbuf.at[slot], xsem.at[slot])

    def o_copy(i, slot, r, c):
        r0 = pl.multiple_of(TS + i * TM, 64)
        return pltpu.make_async_copy(
            obuf.at[slot, pl.ds(r * rs, rs), pl.ds(c * cs, cs)],
            o_hbm.at[pl.ds(r0 + r * rs, rs), pl.ds(c * cs, cs)],
            osem.at[slot])

    def o_wait_all(i, slot):
        r0 = pl.multiple_of(TS + i * TM, 64)
        pltpu.make_async_copy(obuf.at[slot], o_hbm.at[pl.ds(r0, TM)], osem.at[slot]).wait()

    def w_copy(l):
        return pltpu.make_async_copy(w_hbm.at[l], wbuf.at[l], wsem.at[l])

    def w0_quadrant_copy(r, c):
        r0 = pl.multiple_of(r * hd, hd)
        c0 = pl.multiple_of(c * hd, hd)
        return pltpu.make_async_copy(
            w_hbm.at[0, pl.ds(r0, hd), pl.ds(c0, hd)],
            wbuf.at[0, pl.ds(r0, hd), pl.ds(c0, hd)],
            qsem.at[2 * r + c])

    def xs_copy(r0, rows, sem):
        return pltpu.make_async_copy(
            x0_hbm.at[pl.ds(r0, rows)], x0s.at[pl.ds(r0, rows)], ssem.at[sem])

    xa_top = xs_copy(0, TS // 4, 4)
    xa_bot = xs_copy(TS // 4, TS // 4, 5)
    xb_all = xs_copy(TS // 2, TS // 2, 2)
    b_copy = pltpu.make_async_copy(b_hbm, braw, ssem.at[0])
    os_copy = pltpu.make_async_copy(os16, o_hbm.at[pl.ds(0, TS)], ssem.at[3])

    def loop(lo, hi, fn):
        def body(i, carry):
            fn(i)
            return carry
        lax.fori_loop(lo, hi, body, 0)

    b_copy.start()
    xa_bot.start()
    loop(0, 2, lambda r: w0_quadrant_copy(r, 0).start())
    xa_top.start()
    loop(0, 2, lambda r: w0_quadrant_copy(1 - r, 1).start())
    xb_all.start()
    loop(1, n_layers, lambda l: w_copy(l).start())
    x_copy(0, 0).start()

    b_copy.wait()
    bf32[0:n_layers, :] = braw[...].astype(F32)

    def t_index(i1, i2, j):
        return ((i1 - 1) * 7 + i2 - 1) * ntile + j

    def get_t(l, i1, i2, j):
        return pltpu.bitcast(t_ref[l, t_index(i1, i2, j)], BF16)

    def build_t(l, i1):
        for j in range(ntile):
            def w_tile(r, c):
                cols = slice(c * cs + j * LANES, c * cs + (j + 1) * LANES)
                return wbuf[l, r * cs:(r + 1) * cs, cols].astype(F32)
            lvl1 = [_signed_sum([(s, w_tile(*_sub_block(q, k))) for s, q in _RHS[i1]])
                    for k in range(4)]
            for i2 in range(1, 8):
                v = _signed_sum([(s, lvl1[k]) for s, k in _RHS[i2]]).astype(BF16)
                t_ref[l, t_index(i1, i2, j)] = pltpu.bitcast(v, U32)

    def x0_group(u, r, c):
        return x0s[(u * 4 + r) * rh:(u * 4 + r + 1) * rh, c * cs:(c + 1) * cs].astype(F32)

    bias0 = [bf32[0:1, c * cs:(c + 1) * cs] for c in range(4)]
    get_t0 = functools.partial(get_t, 0)
    groups = []
    for u in range(2):
        xg = functools.lru_cache(maxsize=None)(functools.partial(x0_group, u))
        groups.append(_Rows(xg, xg, bias0))
    ga, gb = groups

    def first_product(i1, on):
        build_t(0, i1)
        _outer_product(i1, on, get_t0, wide_order=_FIRST_INNER)

    xa_bot.wait()
    w0_quadrant_copy(0, 0).wait()
    first_product(2, [ga])
    w0_quadrant_copy(1, 0).wait()
    first_product(4, [ga])
    xa_top.wait()
    w0_quadrant_copy(1, 1).wait()
    for i1 in _FIRST_MID:
        first_product(i1, [ga])
    w0_quadrant_copy(0, 1).wait()
    xb_all.wait()
    for i1 in _FIRST_LAST:
        if i1 in (3, 6):
            first_product(i1, [ga, gb])
        else:
            _outer_product(i1, [gb], get_t0, _START_INNER)
    for u in range(2):
        for r in range(4):
            for c in range(4):
                xs32[(u * 4 + r) * rh:(u * 4 + r + 1) * rh, c * cs:(c + 1) * cs] = groups[u].new[r][c]

    def x0_start(r, c):
        return x0s[r * ru:(r + 1) * ru, c * cs:(c + 1) * cs].astype(F32)

    def start_layer(l):
        w_copy(l).wait()
        brow = bf32[pl.ds(l, 1), :]
        xv = [[xs32[r * ru:(r + 1) * ru, c * cs:(c + 1) * cs] for c in range(4)] for r in range(4)]
        new = _cross_layer(
            lambda r, c: xv[r][c], x0_start, [brow[:, c * cs:(c + 1) * cs] for c in range(4)],
            functools.partial(get_t, l), _START_OUTER, _START_INNER,
            before_product=functools.partial(build_t, l))
        for r in range(4):
            for c in range(4):
                xs32[r * ru:(r + 1) * ru, c * cs:(c + 1) * cs] = new[r][c]

    loop(1, n_layers, start_layer)
    os16[...] = xs32[...].astype(BF16)
    os_copy.start()

    def main_block(i):
        slot = i & 1
        x_copy(i, slot).wait()

        @pl.when(i >= 2)
        def _():
            o_wait_all(i - 2, slot)

        @pl.when(i + 1 < n_iter)
        def _():
            x_copy(i + 1, 1 - slot).start()

        x_in = xbuf.at[slot]
        x_out = obuf.at[slot]
        x0v = [[x_in[r * rs:(r + 1) * rs, c * cs:(c + 1) * cs].astype(F32) for c in range(4)]
               for r in range(4)]

        def write_quadrant(q, new):
            for k in (1, 3, 2, 0):
                r, c = _sub_block(q, k)
                x_out[r * rs:(r + 1) * rs, c * cs:(c + 1) * cs] = new[r][c].astype(BF16)
                o_copy(i, slot, r, c).start()

        xv = x0v
        for l in range(n_layers):
            xv = _cross_layer(
                functools.partial(lambda g, r, c: g[r][c], xv), lambda r, c: x0v[r][c],
                [bf32[l:l + 1, c * cs:(c + 1) * cs] for c in range(4)],
                functools.partial(get_t, l), _MAIN_OUTER[l % 6], _MAIN_INNER[l % 6],
                after_quadrant=write_quadrant if l == n_layers - 1 else None)

    loop(0, n_iter, main_block)

    os_copy.wait()
    for i in (n_iter - 2, n_iter - 1):
        o_wait_all(i, i % 2)


@jax.jit
def pallas_standalone__dcn_v2_cross__recsys_kernel(
    x0: jax.Array,
    ws: jax.Array,
    bs: jax.Array,
):
    batch, d = x0.shape
    n_layers = ws.shape[0]
    assert ws.shape == (n_layers, d, d) and bs.shape == (n_layers, d)
    assert (batch - TS) % TM == 0 and (batch - TS) // TM >= 2
    assert d % (4 * LANES) == 0 and 2 <= n_layers <= 8
    ntile = d // 4 // LANES
    return pl.pallas_call(
        _kernel,
        in_specs=[pl.BlockSpec(memory_space=pl.ANY)] * 3,
        out_specs=pl.BlockSpec(memory_space=pl.ANY),
        out_shape=jax.ShapeDtypeStruct((batch, d), x0.dtype),
        scratch_shapes=[
            pltpu.VMEM((2, TM, d), BF16),
            pltpu.VMEM((2, TM, d), BF16),
            pltpu.VMEM((n_layers, d, d), BF16),
            pltpu.VMEM((n_layers, 49 * ntile, d // 8, LANES), U32),
            pltpu.VMEM((n_layers, d), BF16),
            pltpu.VMEM((8, d), F32),
            pltpu.VMEM((TS, d), F32),
            pltpu.VMEM((TS, d), BF16),
            pltpu.VMEM((TS, d), BF16),
            pltpu.SemaphoreType.DMA((2,)),
            pltpu.SemaphoreType.DMA((2,)),
            pltpu.SemaphoreType.DMA((n_layers,)),
            pltpu.SemaphoreType.DMA((6,)),
            pltpu.SemaphoreType.DMA((4,)),
        ],
        compiler_params=pltpu.CompilerParams(
            vmem_limit_bytes=100 * 1024 * 1024,
            disable_bounds_checks=True,
            disable_semaphore_checks=True,
        ),
    )(x0, ws, bs)
```

```python
import functools

import jax
import jax.numpy as jnp
from jax import lax
from jax.experimental import pallas as pl
from jax.experimental.pallas import tpu as pltpu

F32 = jnp.float32
BF16 = jnp.bfloat16
U32 = jnp.uint32

TM = 256
TS = 1024
LANES = 128

_LHS = {1: ((1, 0), (1, 3)), 2: ((1, 2), (1, 3)), 3: ((1, 0),), 4: ((1, 3),),
        5: ((1, 0), (1, 1)), 6: ((1, 2), (-1, 0)), 7: ((1, 1), (-1, 3))}
_RHS = {1: ((1, 0), (1, 3)), 2: ((1, 0),), 3: ((1, 1), (-1, 3)), 4: ((1, 2), (-1, 0)),
        5: ((1, 3),), 6: ((1, 0), (1, 1)), 7: ((1, 2), (1, 3))}
_OUT = {0: {1: 1, 4: 1, 5: -1, 7: 1}, 1: {3: 1, 5: 1}, 2: {2: 1, 4: 1}, 3: {1: 1, 2: -1, 3: 1, 6: 1}}

_MAIN_OUTER = ((3, 6, 5, 2, 1, 4, 7), (4, 3, 1, 2, 5, 7, 6), (3, 5, 6, 2, 1, 4, 7),
               (4, 3, 1, 2, 5, 7, 6), (3, 5, 6, 2, 1, 4, 7), (4, 3, 1, 2, 5, 7, 6))
_MAIN_INNER = (((6, 3, 5, 1, 2, 4, 7), (2, 3, 5, 1, 6, 4, 7)),
               ((6, 3, 5, 1, 2, 4, 7), (2, 3, 5, 1, 6, 4, 7)),
               ((6, 3, 5, 1, 2, 4, 7), (1, 3, 5, 2, 6, 4, 7)),
               ((6, 3, 5, 1, 2, 4, 7), (2, 3, 5, 1, 6, 4, 7)),
               ((6, 3, 5, 1, 2, 4, 7), (2, 3, 6, 4, 1, 5, 7)),
               ((3, 5, 1, 6, 2, 4, 7), (2, 3, 5, 1, 6, 4, 7)))
_START_OUTER = (5, 7, 3, 1, 6, 4, 2)
_START_INNER = ((6, 4, 7, 5, 1, 3, 2), (2, 5, 4, 3, 6, 1, 7))
_FIRST_INNER = (2, 5, 3, 4, 1, 7, 6)
_FIRST_INNER_B = ((7, 4, 1, 5, 3, 6, 2), (2, 5, 4, 6, 3, 1, 7))
_FIRST_MID = (5, 7, 1)
_FIRST_LAST = (4, 7, 3, 2, 6, 5, 1)


def _add(a, b):
    return a + b


def _sub(a, b):
    return a - b


def _zip1(f):
    return lambda a, b: [f(u, v) for u, v in zip(a, b)]


def _signed_sum(terms, add=_add, sub=_sub):
    terms = sorted(terms, key=lambda t: -t[0])
    assert terms[0][0] == 1
    acc = terms[0][1]
    for s, v in terms[1:]:
        acc = add(acc, v) if s == 1 else sub(acc, v)
    return acc


def _sub_block(q, k):
    return 2 * (q // 2) + k // 2, 2 * (q % 2) + k % 2


class _Accumulator:
    def __init__(self, finish, add, sub):
        self.finish, self.add, self.sub = finish, add, sub
        self.pending = {q: [] for q in _OUT}
        self.seen = {q: 0 for q in _OUT}

    def accept(self, i, m):
        for q, coef in _OUT.items():
            if i not in coef:
                continue
            self.pending[q].append((coef[i], m))
            self.seen[q] += 1
            if len(self.pending[q]) == 2:
                self.pending[q] = [(1, _signed_sum(self.pending[q], self.add, self.sub))]
            if self.seen[q] == len(coef):
                self.finish(q, self.pending[q][0][1])


class _Rows:
    def __init__(self, x, x0, bias, after_quadrant=None):
        self.x, self.x0, self.bias, self.after_quadrant = x, x0, bias, after_quadrant
        self.new = [[None] * 4 for _ in range(4)]
        self.acc = _Accumulator(self._finish, _zip1(_zip1(_add)), _zip1(_zip1(_sub)))

    def _finish(self, q, c):
        for k in range(4):
            r, col = _sub_block(q, k)
            y = jnp.concatenate(c[k], axis=1) + self.bias[col]
            self.new[r][col] = self.x0(r, col) * y + self.x(r, col)
        if self.after_quadrant is not None:
            self.after_quadrant(q, self.new)

    def lhs(self, i1, i2):
        return _signed_sum([(s2 * s1, self.x(*_sub_block(q, k)))
                            for s2, k in _LHS[i2] for s1, q in _LHS[i1]])


def _outer_product(i1, groups, get_t, inner_orders=None, wide_order=None):
    ntile = groups[0].bias[0].shape[1] // LANES
    lhs = {}

    def product(j, i2):
        if i2 not in lhs:
            parts = [g.lhs(i1, i2) for g in groups]
            lhs[i2] = (parts[0] if len(parts) == 1 else jnp.concatenate(parts, axis=0)).astype(BF16)
        return jnp.dot(lhs[i2], get_t(i1, i2, j), preferred_element_type=F32)

    out = [[None] * ntile for _ in range(4)]
    if wide_order is not None:
        def finish_wide(k, v):
            out[k] = v
        acc = _Accumulator(finish_wide, _zip1(_add), _zip1(_sub))
        for i2 in wide_order:
            acc.accept(i2, [product(j, i2) for j in range(ntile)])
    else:
        for j in range(ntile):
            def finish(k, v, j=j):
                out[k][j] = v
            acc = _Accumulator(finish, _add, _sub)
            for i2 in inner_orders[j % len(inner_orders)]:
                acc.accept(i2, product(j, i2))
    if len(groups) == 1:
        groups[0].acc.accept(i1, out)
    else:
        n = out[0][0].shape[0] // len(groups)
        for u, g in enumerate(groups):
            g.acc.accept(i1, [[t[u * n:(u + 1) * n] for t in row] for row in out])


def _cross_layer(x, x0, bias, get_t, outer_order, inner_orders,
                 before_product=None, after_quadrant=None):
    g = _Rows(x, x0, bias, after_quadrant)
    for i1 in outer_order:
        if before_product is not None:
            before_product(i1)
        _outer_product(i1, [g], get_t, inner_orders)
    return g.new


def _kernel(x0_hbm, w_hbm, b_hbm, o_hbm,
            xbuf, obuf, wbuf, t_ref, braw, bf32, xs32, x0s, os16,
            xsem, osem, wsem, ssem, qsem):
    n_layers, d, _ = wbuf.shape
    n_iter = (x0_hbm.shape[0] - TS) // TM
    cs = d // 4
    hd = d // 2
    ntile = cs // LANES
    rs = TM // 4
    ru = TS // 4
    rh = TS // 8

    def x_copy(i, slot):
        r0 = pl.multiple_of(TS + i * TM, 64)
        return pltpu.make_async_copy(x0_hbm.at[pl.ds(r0, TM)], xbuf.at[slot], xsem.at[slot])

    def o_copy(i, slot, r, c):
        r0 = pl.multiple_of(TS + i * TM, 64)
        return pltpu.make_async_copy(
            obuf.at[slot, pl.ds(r * rs, rs), pl.ds(c * cs, cs)],
            o_hbm.at[pl.ds(r0 + r * rs, rs), pl.ds(c * cs, cs)],
            osem.at[slot])

    def o_wait_all(i, slot):
        r0 = pl.multiple_of(TS + i * TM, 64)
        pltpu.make_async_copy(obuf.at[slot], o_hbm.at[pl.ds(r0, TM)], osem.at[slot]).wait()

    def w_copy(l):
        return pltpu.make_async_copy(w_hbm.at[l], wbuf.at[l], wsem.at[l])

    def w0_quadrant_copy(r, c):
        r0 = pl.multiple_of(r * hd, hd)
        c0 = pl.multiple_of(c * hd, hd)
        return pltpu.make_async_copy(
            w_hbm.at[0, pl.ds(r0, hd), pl.ds(c0, hd)],
            wbuf.at[0, pl.ds(r0, hd), pl.ds(c0, hd)],
            qsem.at[2 * r + c])

    def xs_copy(r0, rows, sem):
        return pltpu.make_async_copy(
            x0_hbm.at[pl.ds(r0, rows)], x0s.at[pl.ds(r0, rows)], ssem.at[sem])

    xa_top = xs_copy(0, TS // 4, 4)
    xa_bot = xs_copy(TS // 4, TS // 4, 5)
    xb_all = xs_copy(TS // 2, TS // 2, 2)
    b_copy = pltpu.make_async_copy(b_hbm, braw, ssem.at[0])
    os_copy = pltpu.make_async_copy(os16, o_hbm.at[pl.ds(0, TS)], ssem.at[3])

    def loop(lo, hi, fn):
        def body(i, carry):
            fn(i)
            return carry
        lax.fori_loop(lo, hi, body, 0)

    b_copy.start()
    xa_bot.start()
    loop(0, 2, lambda r: w0_quadrant_copy(r, 0).start())
    xa_top.start()
    loop(0, 2, lambda r: w0_quadrant_copy(1 - r, 1).start())
    xb_all.start()
    loop(1, n_layers, lambda l: w_copy(l).start())
    x_copy(0, 0).start()

    b_copy.wait()
    bf32[0:n_layers, :] = braw[...].astype(F32)

    def t_index(i1, i2, j):
        return ((i1 - 1) * 7 + i2 - 1) * ntile + j

    def get_t(l, i1, i2, j):
        return pltpu.bitcast(t_ref[l, t_index(i1, i2, j)], BF16)

    def build_t(l, i1):
        for j in range(ntile):
            def w_tile(r, c):
                cols = slice(c * cs + j * LANES, c * cs + (j + 1) * LANES)
                return wbuf[l, r * cs:(r + 1) * cs, cols].astype(F32)
            lvl1 = [_signed_sum([(s, w_tile(*_sub_block(q, k))) for s, q in _RHS[i1]])
                    for k in range(4)]
            for i2 in range(1, 8):
                v = _signed_sum([(s, lvl1[k]) for s, k in _RHS[i2]]).astype(BF16)
                t_ref[l, t_index(i1, i2, j)] = pltpu.bitcast(v, U32)

    def x0_group(u, r, c):
        return x0s[(u * 4 + r) * rh:(u * 4 + r + 1) * rh, c * cs:(c + 1) * cs].astype(F32)

    bias0 = [bf32[0:1, c * cs:(c + 1) * cs] for c in range(4)]
    get_t0 = functools.partial(get_t, 0)
    groups = []
    for u in range(2):
        xg = functools.lru_cache(maxsize=None)(functools.partial(x0_group, u))
        groups.append(_Rows(xg, xg, bias0))
    ga, gb = groups

    def first_product(i1, on):
        build_t(0, i1)
        _outer_product(i1, on, get_t0, wide_order=_FIRST_INNER)

    xa_bot.wait()
    w0_quadrant_copy(0, 0).wait()
    first_product(2, [ga])
    w0_quadrant_copy(1, 0).wait()
    first_product(4, [ga])
    xa_top.wait()
    w0_quadrant_copy(1, 1).wait()
    for i1 in _FIRST_MID:
        first_product(i1, [ga])
    w0_quadrant_copy(0, 1).wait()
    xb_all.wait()
    for i1 in _FIRST_LAST:
        if i1 in (3, 6):
            first_product(i1, [ga, gb])
        else:
            _outer_product(i1, [gb], get_t0, _FIRST_INNER_B)
    for u in range(2):
        for r in range(4):
            for c in range(4):
                xs32[(u * 4 + r) * rh:(u * 4 + r + 1) * rh, c * cs:(c + 1) * cs] = groups[u].new[r][c]

    def x0_start(r, c):
        return x0s[r * ru:(r + 1) * ru, c * cs:(c + 1) * cs].astype(F32)

    def start_layer(l):
        w_copy(l).wait()
        brow = bf32[pl.ds(l, 1), :]
        xv = [[xs32[r * ru:(r + 1) * ru, c * cs:(c + 1) * cs] for c in range(4)] for r in range(4)]
        new = _cross_layer(
            lambda r, c: xv[r][c], x0_start, [brow[:, c * cs:(c + 1) * cs] for c in range(4)],
            functools.partial(get_t, l), _START_OUTER, _START_INNER,
            before_product=functools.partial(build_t, l))
        for r in range(4):
            for c in range(4):
                xs32[r * ru:(r + 1) * ru, c * cs:(c + 1) * cs] = new[r][c]
                os16[r * ru:(r + 1) * ru, c * cs:(c + 1) * cs] = new[r][c].astype(BF16)

    loop(1, n_layers, start_layer)
    os_copy.start()

    def main_block(i):
        slot = i & 1
        x_copy(i, slot).wait()

        @pl.when(i >= 2)
        def _():
            o_wait_all(i - 2, slot)

        @pl.when(i + 1 < n_iter)
        def _():
            x_copy(i + 1, 1 - slot).start()

        x_in = xbuf.at[slot]
        x_out = obuf.at[slot]
        x0v = [[x_in[r * rs:(r + 1) * rs, c * cs:(c + 1) * cs].astype(F32) for c in range(4)]
               for r in range(4)]

        def write_quadrant(q, new):
            for k in (1, 3, 2, 0):
                r, c = _sub_block(q, k)
                x_out[r * rs:(r + 1) * rs, c * cs:(c + 1) * cs] = new[r][c].astype(BF16)
                o_copy(i, slot, r, c).start()

        xv = x0v
        for l in range(n_layers):
            xv = _cross_layer(
                functools.partial(lambda g, r, c: g[r][c], xv), lambda r, c: x0v[r][c],
                [bf32[l:l + 1, c * cs:(c + 1) * cs] for c in range(4)],
                functools.partial(get_t, l), _MAIN_OUTER[l % 6], _MAIN_INNER[l % 6],
                after_quadrant=write_quadrant if l == n_layers - 1 else None)

    loop(0, n_iter, main_block)

    os_copy.wait()
    for i in (n_iter - 2, n_iter - 1):
        o_wait_all(i, i % 2)


@jax.jit
def pallas_standalone__dcn_v2_cross__recsys_kernel(
    x0: jax.Array,
    ws: jax.Array,
    bs: jax.Array,
):
    batch, d = x0.shape
    n_layers = ws.shape[0]
    assert ws.shape == (n_layers, d, d) and bs.shape == (n_layers, d)
    assert (batch - TS) % TM == 0 and (batch - TS) // TM >= 2
    assert d % (4 * LANES) == 0 and 2 <= n_layers <= 8
    ntile = d // 4 // LANES
    return pl.pallas_call(
        _kernel,
        in_specs=[pl.BlockSpec(memory_space=pl.ANY)] * 3,
        out_specs=pl.BlockSpec(memory_space=pl.ANY),
        out_shape=jax.ShapeDtypeStruct((batch, d), x0.dtype),
        scratch_shapes=[
            pltpu.VMEM((2, TM, d), BF16),
            pltpu.VMEM((2, TM, d), BF16),
            pltpu.VMEM((n_layers, d, d), BF16),
            pltpu.VMEM((n_layers, 49 * ntile, d // 8, LANES), U32),
            pltpu.VMEM((n_layers, d), BF16),
            pltpu.VMEM((8, d), F32),
            pltpu.VMEM((TS, d), F32),
            pltpu.VMEM((TS, d), BF16),
            pltpu.VMEM((TS, d), BF16),
            pltpu.SemaphoreType.DMA((2,)),
            pltpu.SemaphoreType.DMA((2,)),
            pltpu.SemaphoreType.DMA((n_layers,)),
            pltpu.SemaphoreType.DMA((6,)),
            pltpu.SemaphoreType.DMA((4,)),
        ],
        compiler_params=pltpu.CompilerParams(
            vmem_limit_bytes=100 * 1024 * 1024,
            disable_bounds_checks=True,
            disable_semaphore_checks=True,
        ),
    )(x0, ws, bs)
```
